```python
import os as _os
_os.environ.setdefault("JAX_PLATFORMS", "cpu")
import jax
import jax.numpy as jnp

def _softmax(x, axis=-1):
    return jax.nn.softmax(x, axis=axis)
def _gelu(x):
    return jax.nn.gelu(x, approximate=True)
def _silu(x):
    return jax.nn.silu(x)
def _sigmoid(x):
    return jax.nn.sigmoid(x)
def _layernorm(x, axis=-1, eps=1e-5):
    m = jnp.mean(x, axis=axis, keepdims=True)
    v = jnp.var(x, axis=axis, keepdims=True)
    return (x - m) / jnp.sqrt(v + eps)
def _scatter_add(tgt, idx, src, axis=0):
    return tgt.at[idx].add(src)
def _segment_sum(src, seg, n):
    return jax.ops.segment_sum(src, seg, n)
class _Rng:
    def __init__(self, key):
        self._k = key
    def _next(self):
        self._k, sub = jax.random.split(self._k)
        return sub
    def normal(self, shape):
        return jax.random.normal(self._next(), shape, dtype=jnp.bfloat16)
    def randint(self, lo, hi, shape):
        return jax.random.randint(self._next(), shape, lo, hi, dtype=jnp.int32)
    def uniform(self, shape, lo=0.0, hi=1.0):
        return jax.random.uniform(self._next(), shape, jnp.bfloat16, lo, hi)
    def permutation(self, n):
        return jax.random.permutation(self._next(), n)


kernel_name = 'concat_heads__gqa_block_cached__mha_block_cached__near_ridge'

def setup_inputs():
    _rng = _Rng(jax.random.key(int.from_bytes(__import__("os").urandom(4), "little")))
    _w = (lambda a: (lambda t: t.astype(jnp.bfloat16) if jnp.issubdtype(t.dtype, jnp.floating) else t)(jnp.asarray(a)))
    def _A_setup():
        B, Sq, D = 8, 112, 448
        Hq, Hkv, Sk, Dh = 16, 8, 512, 256
        assert Hq % Hkv == 0, (Hq, Hkv)
        return {
            "x": _w((lambda *s: _rng.normal(s) * 0.8)(B, Sq, D)),
            "k_cache": _w((lambda *s: _rng.normal(s) * 0.8)(B, Hkv, Sk, Dh)),
            "v_cache": _w((lambda *s: _rng.normal(s) * 0.05)(B, Hkv, Sk, Dh)),
            "wq": _w((lambda *s: _rng.normal(s) * 0.8)(D, Hq * Dh) * (D ** -0.5)),
            "wo": _w((lambda *s: _rng.normal(s) * 0.05)(Hq * Dh, D) * ((Hq * Dh) ** -0.5)),
        }
    _A_in = _A_setup()

    def _B_setup():
        B, Sq, D = 8, 112, 448
        H, Sk, Dh = 16, 512, 256
        return {
            "x": _w((lambda *s: _rng.normal(s) * 0.8)(B, Sq, D)),
            "k_cache": _w((lambda *s: _rng.normal(s) * 0.8)(B, H, Sk, Dh)),
            "v_cache": _w((lambda *s: _rng.normal(s) * 0.05)(B, H, Sk, Dh)),
            "wq": _w((lambda *s: _rng.normal(s) * 0.8)(D, H * Dh) * (D ** -0.5)),
            "wo": _w((lambda *s: _rng.normal(s) * 0.05)(H * Dh, D) * ((H * Dh) ** -0.5)),
        }
    _B_in = _B_setup()

    return {
        "A_x": _A_in["x"],
        "A_k_cache": _A_in["k_cache"],
        "A_v_cache": _A_in["v_cache"],
        "A_wq": _A_in["wq"],
        "A_wo": _A_in["wo"],
        "B_x": _B_in["x"],
        "B_k_cache": _B_in["k_cache"],
        "B_v_cache": _B_in["v_cache"],
        "B_wq": _B_in["wq"],
        "B_wo": _B_in["wo"],
    }

def reference(A_x, A_k_cache, A_v_cache, A_wq, A_wo, B_x, B_k_cache, B_v_cache, B_wq, B_wo):
    def _A_ref(x, k_cache, v_cache, wq, wo):
        B, Sq, D = x.shape
        Hq, Dh = 16, 256
        Hkv = k_cache.shape[1]
        rep = Hq // Hkv
        q = (lambda x, *d: x.transpose(*d))((x @ wq).reshape(B, Sq, Hq, Dh), 0, 2, 1, 3)
        k = jnp.repeat(k_cache, rep, axis=1)
        v = jnp.repeat(v_cache, rep, axis=1)
        scores = jnp.einsum("bhqd,bhkd->bhqk", q, k) * (Dh ** -0.5)
        p = _softmax(scores, axis=-1)
        o = jnp.einsum("bhqk,bhkd->bhqd", p, v)
        return (lambda x, *d: x.transpose(*d))(o, 0, 2, 1, 3).reshape(B, Sq, Hq * Dh) @ wo

    def _B_ref(x, k_cache, v_cache, wq, wo):
        B, Sq, D = x.shape
        H, Dh = 16, 256
        q = (lambda x, *d: x.transpose(*d))((x @ wq).reshape(B, Sq, H, Dh), 0, 2, 1, 3)
        scores = jnp.einsum("bhqd,bhkd->bhqk", q, k_cache) * (Dh ** -0.5)
        p = _softmax(scores, axis=-1)
        o = jnp.einsum("bhqk,bhkd->bhqd", p, v_cache)
        return (lambda x, *d: x.transpose(*d))(o, 0, 2, 1, 3).reshape(B, Sq, H * Dh) @ wo

    a = _A_ref(A_x, A_k_cache, A_v_cache, A_wq, A_wo)
    b = _B_ref(B_x, B_k_cache, B_v_cache, B_wq, B_wo)
    return jnp.concatenate([a, b], axis=-1)
```

```python
import jax, jax.numpy as jnp
import jax.experimental.pallas as pl
import jax.experimental.pallas.tpu as pltpu
import math

B, SQ, D, H, HKV, SK, DH = 8, 112, 448, 16, 8, 512, 256
G = 8
GW = 2 * DH
NP = 512
QSCALE = (DH ** -0.5) * math.log2(math.e)
NBS = 16
NODMA = 0
P0 = 4
SEG_A = [(0,4,1),(4,8,2),(8,32,4)]
SEG_B = [(0,24,4),(24,28,2),(28,32,1)]
bf16 = jnp.bfloat16
f32 = jnp.float32

S_XA = 0
S_XB = 4
S_W = 5
S_A = S_W + 32
S_B = S_A + 64
S_O = S_B + 2 * NBS
NSEM = S_O + 4

def dot_nn(a, b):
    return jnp.dot(a, b, preferred_element_type=f32)
def dot_nt(a, b):
    return jax.lax.dot_general(a, b, (((1,), (1,)), ((), ())), preferred_element_type=f32)

def softmax_parts(s):
    m = jnp.max(s, axis=-1, keepdims=True)
    p = jnp.exp2(s - m)
    l = jnp.sum(p, axis=-1, keepdims=True)
    return p.astype(bf16), 1.0 / l

def isint(x): return isinstance(x, (int, bool))
def land(a, b):
    if isint(a): return b if a else False
    if isint(b): return a if b else False
    return jnp.logical_and(a, b)

def kernel(ax, ak, av, awq, awo, bx, bk, bv, bwq, bwo, out,
           xbuf, wqbuf, wobuf, kab, vab, kbb, vbb, acc, obuf, sem):
    def mo(x, m):
        return x if isint(x) else pl.multiple_of(x, m)
    def xa_copy(bp):
        r = pl.ds(mo(bp * 2 * SQ, 16), 2 * SQ)
        return pltpu.make_async_copy(ax.at[r], xbuf.at[0, r], sem.at[S_XA + bp])
    def xb_copy():
        return pltpu.make_async_copy(bx, xbuf.at[1], sem.at[S_XB])
    def col(j):
        return pl.ds(mo(j * GW, GW), GW)
    def wq_copy(br, j):
        return pltpu.make_async_copy((awq, bwq)[br].at[:, col(j)], wqbuf.at[br, j], sem.at[S_W + br * 16 + j])
    def wo_copy(br, j):
        off = 0 if br == 0 else NP - D
        return pltpu.make_async_copy((awo, bwo)[br].at[:, col(j)], wobuf.at[br, j, pl.ds(off, D)], sem.at[S_W + br * 16 + 8 + j])
    def a_copies(j, bp):
        t = j * 4 + bp
        return [pltpu.make_async_copy(ak.at[pl.ds(2 * bp, 2), j], kab.at[t], sem.at[S_A + 2 * t]),
                pltpu.make_async_copy(av.at[pl.ds(2 * bp, 2), j], vab.at[t], sem.at[S_A + 2 * t + 1])]
    def b_copies(j, bp):
        slot = (j * 4 + bp) & (NBS - 1)
        return [pltpu.make_async_copy(bk.at[pl.ds(2 * bp, 2), pl.ds(2 * j, 2)], kbb.at[slot], sem.at[S_B + 2 * slot]),
                pltpu.make_async_copy(bv.at[pl.ds(2 * bp, 2), pl.ds(2 * j, 2)], vbb.at[slot], sem.at[S_B + 2 * slot + 1])]
    def o_copy(bp):
        r = pl.ds(mo(bp * 2 * SQ, 16), 2 * SQ)
        return pltpu.make_async_copy(obuf.at[r], out.at[r], sem.at[S_O + bp])
    def start(c):
        if not NODMA: c.start()
    def wait(c):
        if not NODMA: c.wait()
    def when(cond, fn):
        if isint(cond):
            if cond: fn()
        else:
            pl.when(cond)(fn)

    def issue_pkg(p, lo=0, hi=64, limit=32 + NBS):
        j = (p >> 2) & 7
        bp = p & 3
        first = bp == 0
        if lo < 32:
            is_a = True if hi <= 32 else p < 32
            if isint(p) and p < 4:
                start(xa_copy(p))
            when(land(is_a, first), lambda: start(wq_copy(0, j)))
            when(is_a, lambda: [start(c) for c in a_copies(j, bp)] and None)
            when(land(is_a, first), lambda: start(wo_copy(0, j)))
        if hi > 32 and lo < limit:
            is_b = land(True if lo >= 32 else p >= 32, True if hi <= limit else p < limit)
            if lo <= 32: when(p == 32, lambda: start(xb_copy()))
            when(land(is_b, first), lambda: start(wq_copy(1, j)))
            when(is_b, lambda: [start(c) for c in b_copies(j, bp)] and None)
            when(land(is_b, first), lambda: start(wo_copy(1, j)))

    for p in range(P0):
        issue_pkg(p, p, p + 1)
    acc[...] = jnp.zeros_like(acc)
    for j in range(G):
        wobuf[0, j, D:NP, :] = jnp.zeros((NP - D, GW), bf16)
        wobuf[1, j, 0:NP - D, :] = jnp.zeros((NP - D, GW), bf16)

    def rows(b):
        return pl.ds(mo(b * SQ, 16), SQ)
    def qproj(br, j, b):
        return (dot_nn(xbuf[br, rows(b), :], wqbuf[br, j]) * QSCALE).astype(bf16)

    def a_waits(j, bp, lo):
        if lo < 4: when(j == 0, lambda: wait(xa_copy(bp)))
        when(bp == 0, lambda: (wait(wq_copy(0, j)), wait(wo_copy(0, j))) and None)
        for c in a_copies(j, bp): wait(c)

    def a_compute(j, bp, lo, hi):
        t = j * 4 + bp
        for c in range(2):
            issue_pkg(P0 + 2 * t + c, P0 + 2 * lo + c, P0 + 2 * (hi - 1) + c + 1)
        q = [qproj(0, j, 2 * bp + i) for i in range(2)]
        s = [dot_nt(jnp.concatenate([q[i][:, :DH], q[i][:, DH:]], axis=0), kab[t, i]) for i in range(2)]
        sm = [softmax_parts(s[i]) for i in range(2)]
        o = [(dot_nn(sm[i][0], vab[t, i]) * sm[i][1]).astype(bf16) for i in range(2)]
        for i in range(2):
            oc = jnp.concatenate([o[i][:SQ], o[i][SQ:]], axis=1)
            acc[rows(2 * bp + i), 0:NP] += dot_nt(oc, wobuf[0, j])

    def b_waits(j, bp, lo):
        when(bp == 0, lambda: (wait(wq_copy(1, j)), wait(wo_copy(1, j))) and None)
        for c in b_copies(j, bp): wait(c)

    def b_compute(j, bp, lo, hi):
        t = j * 4 + bp
        slot = t & (NBS - 1)
        if lo - 1 + NBS < 32:
            p = 32 + t - 1 + NBS
            if lo == 0:
                when(t > 0, lambda: issue_pkg(p, 32 + NBS, 32 + hi - 1 + NBS, 64))
            else:
                issue_pkg(p, 32 + lo - 1 + NBS, 32 + hi - 1 + NBS, 64)
        q = [qproj(1, j, 2 * bp + i) for i in range(2)]
        s = [[dot_nt(q[i][:, h * DH:(h + 1) * DH], kbb[slot, i, h]) for h in range(2)] for i in range(2)]
        sm = [[softmax_parts(s[i][h]) for h in range(2)] for i in range(2)]
        o = [[(dot_nn(sm[i][h][0], vbb[slot, i, h]) * sm[i][h][1]).astype(bf16) for h in range(2)] for i in range(2)]
        c0 = 2 * D - NP
        last = hi > 28
        for i in range(2):
            r = rows(2 * bp + i)
            new = acc[r, c0:c0 + NP] + dot_nt(jnp.concatenate(o[i], axis=1), wobuf[1, j])
            acc[r, c0:c0 + NP] = new
            if last:
                obuf[r, 0:c0] = acc[r, 0:c0].astype(bf16)
                obuf[r, c0:c0 + NP] = new.astype(bf16)
        if last:
            when(j == G - 1, lambda: o_copy(bp).start())

    def run_segment(waits, compute, lo, hi, U):
        n = (hi - lo) // U
        def body(i, carry):
            its = []
            for u in range(U):
                if U == 4:
                    j, bp = lo // 4 + i, u
                else:
                    t = lo + i * U + u
                    j = t >> 2
                    bp = (t & 3) if U == 1 else ((lo + i * U) & 3) + u
                its.append((j, bp))
            for j, bp in its: waits(j, bp, lo)
            for j, bp in its: compute(j, bp, lo, hi)
            return carry
        if n == 1:
            body(0, 0)
        else:
            jax.lax.fori_loop(0, n, body, 0)

    for lo, hi, U in SEG_A:
        run_segment(a_waits, a_compute, lo, hi, U)
    wait(xb_copy())
    for lo, hi, U in SEG_B:
        run_segment(b_waits, b_compute, lo, hi, U)
    for bp in range(4):
        o_copy(bp).wait()

@jax.jit
def pallas_concat_heads__gqa_block_cached__mha_block_cached__near_ridge_kernel(A_x, A_k_cache, A_v_cache, A_wq, A_wo, B_x, B_k_cache, B_v_cache, B_wq, B_wo):
    ax = A_x.reshape(B*SQ, D); bx = B_x.reshape(B*SQ, D)
    hbm = pl.BlockSpec(memory_space=pltpu.HBM)
    out = pl.pallas_call(
        kernel,
        in_specs=[hbm] * 10,
        out_specs=hbm,
        out_shape=jax.ShapeDtypeStruct((B*SQ, 2*D), bf16),
        scratch_shapes=[
            pltpu.VMEM((2, B*SQ, D), bf16),
            pltpu.VMEM((2, G, D, GW), bf16),
            pltpu.VMEM((2, G, NP, GW), bf16),
            pltpu.VMEM((32, 2, SK, DH), bf16),
            pltpu.VMEM((32, 2, SK, DH), bf16),
            pltpu.VMEM((NBS, 2, 2, SK, DH), bf16),
            pltpu.VMEM((NBS, 2, 2, SK, DH), bf16),
            pltpu.VMEM((B*SQ, 2*D), f32),
            pltpu.VMEM((B*SQ, 2*D), bf16),
            pltpu.SemaphoreType.DMA((NSEM,)),
        ],
        compiler_params=pltpu.CompilerParams(vmem_limit_bytes=110*1024*1024, disable_bounds_checks=True),
    )(ax, A_k_cache, A_v_cache, A_wq, A_wo.T, bx, B_k_cache, B_v_cache, B_wq, B_wo.T)
    return out.reshape(B, SQ, 2*D)
```

```python
import jax, jax.numpy as jnp
import jax.experimental.pallas as pl
import jax.experimental.pallas.tpu as pltpu
import math

B, SQ, D, H, HKV, SK, DH = 8, 112, 448, 16, 8, 512, 256
M = B * SQ
G = 8
GW = 2 * DH
NP = 512
C0 = 2 * D - NP
QSCALE = (DH ** -0.5) * math.log2(math.e)
NBS = 16
NODMA = 0
SCOPES = 0
P0 = 4
V2LO = 13
TPOS = 'q'
TSCHED = [[], [0], [1, 2], [3], [4, 5, 6]]
bf16 = jnp.bfloat16
f32 = jnp.float32

S_XA = 0
S_XB = 4
S_W = 5
S_KV = S_W + 32
S_V31 = S_KV + 2 * (32 + NBS)
S_O = S_V31 + 1
NSEM = S_O + 5

def dot_nn(a, b):
    return jnp.dot(a, b, preferred_element_type=f32)
def dot_nt(a, b):
    return jax.lax.dot_general(a, b, (((1,), (1,)), ((), ())), preferred_element_type=f32)

def softmax_parts(s):
    m = jnp.max(s, axis=-1, keepdims=True)
    p = jnp.exp2(s - m)
    l = jnp.sum(p, axis=-1, keepdims=True)
    return p.astype(bf16), 1.0 / l

def isint(x): return isinstance(x, (int, bool))
def land(a, b):
    if isint(a): return b if a else False
    if isint(b): return a if b else False
    return jnp.logical_and(a, b)
def sel(c, a, b):
    if isint(c): return a if c else b
    return jnp.where(c, a, b)

class _NoScope:
    def __enter__(self): return None
    def __exit__(self, *a): return False
def scope(name):
    return jax.named_scope(name) if SCOPES else _NoScope()

def kernel(ax, ak, av, awq, awo, bx, bk, bv, bwq, bwo, out,
           xbuf, wqbuf, wobuf, wolast, kbuf, vbuf, accT, accR, oscr, obuf, sem):
    def mo(x, m):
        return x if isint(x) else pl.multiple_of(x, m)
    def xa_copy(bp):
        r = pl.ds(bp * 2 * SQ, 2 * SQ)
        return pltpu.make_async_copy(ax.at[r], xbuf.at[0, r], sem.at[S_XA + bp])
    def xb_copy():
        return pltpu.make_async_copy(bx, xbuf.at[1], sem.at[S_XB])
    def col(j):
        return pl.ds(mo(j * GW, GW), GW)
    def wq_copy(br, j):
        return pltpu.make_async_copy((awq, bwq)[br].at[:, col(j)], wqbuf.at[br * G + j], sem.at[S_W + br * G + j])
    def wo_copy(br, j):
        if br == 1 and isint(j) and j == G - 1:
            dst = wolast.at[pl.ds(NP - D, D)]
        else:
            dst = wobuf.at[br * G + j]
        return pltpu.make_async_copy((awo, bwo)[br].at[:, col(j)], dst, sem.at[S_W + 16 + br * G + j])
    def a_copies(j, bp):
        t = j * 4 + bp
        return [pltpu.make_async_copy(src.at[2 * bp + i, j], buf.at[t, pl.ds(i * SK, SK)], sem.at[S_KV + 2 * t + kv])
                for kv, (src, buf) in enumerate(((ak, kbuf), (av, vbuf))) for i in range(2)]
    def a_waits(j, bp):
        t = j * 4 + bp
        return [pltpu.make_async_copy(buf.at[t], buf.at[t], sem.at[S_KV + 2 * t + kv]) for kv, buf in enumerate((kbuf, vbuf))]
    def b_copies(j, bp):
        slot = (j * 4 + bp) & (NBS - 1)
        s0 = S_KV + 64 + 2 * slot
        dst = pl.ds(32 + 2 * slot, 2)
        ck = pltpu.make_async_copy(bk.at[pl.ds(2 * bp, 2), j], kbuf.at[dst], sem.at[s0])
        if isint(j) and j == G - 1 and bp == 3:
            return [ck] + [pltpu.make_async_copy(bv.at[2 * bp + i, j], vbuf.at[32 + 2 * slot + i],
                                                 sem.at[(s0 + 1, S_V31)[i]]) for i in range(2)]
        return [ck, pltpu.make_async_copy(bv.at[pl.ds(2 * bp, 2), j], vbuf.at[dst], sem.at[s0 + 1])]
    def o_copy(k):
        r = pl.ds(k * 2 * SQ, 2 * SQ) if k < 3 else pl.ds((k + 3) * SQ, SQ)
        return pltpu.make_async_copy(obuf.at[r], out.at[r], sem.at[S_O + k])
    def start(c):
        if not NODMA: c.start()
    def wait(c):
        if not NODMA: c.wait()
    def when(cond, fn):
        if isint(cond):
            if cond: fn()
        else:
            pl.when(cond)(fn)

    def issue_pkg(gi, bp, ok):
        first = bp == 0
        j = gi & (G - 1)
        def fa():
            if isint(gi) and gi == 0: start(xa_copy(bp))
            if first: start(wq_copy(0, j))
            for c in a_copies(j, bp): start(c)
            if first: start(wo_copy(0, j))
        when(land(ok, gi < G), fa)
        if first: when(land(ok, gi == G), lambda: start(xb_copy()))
        def fb(j):
            if first: start(wq_copy(1, j))
            for c in b_copies(j, bp): start(c)
            if first: start(wo_copy(1, j))
        if isint(gi) or bp in (1, 2):
            when(land(ok, gi >= G), lambda: fb(j))
        else:
            when(land(ok, land(gi >= G, gi < 2 * G - 1)), lambda: fb(j))
            when(land(ok, gi == 2 * G - 1), lambda: fb(G - 1))

    def issue(gi, k):
        for c in range(2):
            p = P0 + 2 * k + c
            g = 2 * gi + p // 4
            if isint(gi) and gi >= G: continue
            issue_pkg(g, p % 4, g < G + NBS // 4)
        g = gi + NBS // 4
        if not (isint(gi) and gi < G):
            issue_pkg(g, k, land(gi >= G, g < 2 * G))

    def rows(b):
        return pl.ds(b * SQ, SQ)
    def qproj(gi, b):
        return (dot_nn(xbuf[gi >> 3, rows(b), :], wqbuf[gi]) * QSCALE).astype(bf16)
    def blk(buf, gi, bp, i, h):
        is_a = gi < G
        t = (gi & (G - 1)) * 4 + bp
        pair = sel(is_a, t, 32 + 2 * (t & (NBS - 1)) + i)
        half = sel(is_a, i, h)
        return buf[pair, pl.ds(mo(half * SK, SK), SK), :]
    def scores(gi, bp, i, q):
        return [softmax_parts(dot_nt(q[:, h * DH:(h + 1) * DH], blk(kbuf, gi, bp, i, h))) for h in range(2)]
    def pv(gi, bp, i, sm):
        return jnp.concatenate([(dot_nn(sm[h][0], blk(vbuf, gi, bp, i, h)) * sm[h][1]).astype(bf16) for h in range(2)], axis=1)
    def oproj_t(gi, n):
        c = slice(n * 128, (n + 1) * 128)
        r = pl.ds(mo((gi >> 3) * D, 8), D)
        y = dot_nt(wobuf[gi], oscr[c, :])
        if isint(gi) and gi == 0:
            accT[r, c] = y
        else:
            accT[r, c] += y
    def xpose(n, mlo, mhi):
        accR[n * 128:(n + 1) * 128, mlo * 128:mhi * 128] = accT[mlo * 128:mhi * 128, n * 128:(n + 1) * 128].T

    def waits(gi, bps):
      with scope("w"):
        j = gi & (G - 1)
        def wa():
            for bp in bps:
                if isint(gi) and gi == 0: wait(xa_copy(bp))
                if bp == 0:
                    wait(wq_copy(0, j)); wait(wo_copy(0, j))
                for c in a_waits(j, bp): wait(c)
        def wb():
            for bp in bps:
                if bp == 0:
                    wait(wq_copy(1, j)); wait(wo_copy(1, j))
                for c in b_copies(j, bp): wait(c)
        when(gi < G, wa)
        if 0 in bps: when(gi == G, lambda: wait(xb_copy()))
        when(gi >= G, wb)

    def group(gi, wp, extra=None):
        for bp in range(4):
            if bp in wp:
                nxt = min([w for w in wp if w > bp] + [4])
                waits(gi, range(bp, nxt))
            q = [qproj(gi, 2 * bp + i) for i in range(2)]
            if TPOS == "q":
                for n in TSCHED[bp]: oproj_t(gi, n)
            if extra is not None: extra(bp)
            sm = [scores(gi, bp, i, q[i]) for i in range(2)]
            if TPOS == "s":
                for n in TSCHED[bp]: oproj_t(gi, n)
            for i in range(2):
                oscr[rows(2 * bp + i), :] = pv(gi, bp, i, sm[i])
            issue(gi, bp)
        for n in TSCHED[4]: oproj_t(gi, n)

    for p in range(P0):
        issue_pkg(p // 4, p % 4, True)
    wolast[0:NP - D, :] = jnp.zeros((NP - D, GW), bf16)

    def zero_b(bp):
        accT[D + bp * SQ:D + (bp + 1) * SQ, :] = jnp.zeros((SQ, M), f32)
    with scope("g0"):
        group(0, (0, 1, 2, 3), zero_b)

    def xpose_a(bp):
        for n in ((0, 1), (2, 3), (4, 5), (6,))[bp]: xpose(n, 0, 3)
    def body(gi, carry):
        fine = jnp.logical_or(gi == 1, gi >= V2LO)
        @pl.when(fine)
        def _():
            with scope("v2"):
                group(gi, (0, 2), xpose_a)
        @pl.when(jnp.logical_not(fine))
        def _():
            with scope("v1"):
                group(gi, (0,))
        return carry
    jax.lax.fori_loop(1, 2 * G - 1, body, 0)

    gi = 2 * G - 1
    def finish(b, o):
        r = rows(b)
        obuf[r, 0:C0] = accR[r, 0:C0].astype(bf16)
        obuf[r, C0:2 * D] = (accR[r, C0:2 * D] + dot_nt(o, wolast[...])).astype(bf16)
    with scope("last"):
        for bp in range(3):
            waits(gi, [bp])
            q = [qproj(gi, 2 * bp + i) for i in range(2)]
            for n in (2 * bp, 2 * bp + 1): xpose(n, 3, 7)
            sm = [scores(gi, bp, i, q[i]) for i in range(2)]
            o = [pv(gi, bp, i, sm[i]) for i in range(2)]
            for i in range(2): finish(2 * bp + i, o[i])
            if bp == 2:
                q = [qproj(gi, 6 + i) for i in range(2)]
                xpose(6, 3, 7)
            o_copy(bp).start()
        ck, cv0, cv1 = b_copies(G - 1, 3)
        with scope("wk"): wait(ck)
        sm = [scores(gi, 3, i, q[i]) for i in range(2)]
        for i, c in enumerate((cv0, cv1)):
            with scope("wv"): wait(c)
            finish(6 + i, pv(gi, 3, i, sm[i]))
            o_copy(3 + i).start()
    for k in range(5):
        with scope("wo"): o_copy(k).wait()

@jax.jit
def pallas_concat_heads__gqa_block_cached__mha_block_cached__near_ridge_kernel(A_x, A_k_cache, A_v_cache, A_wq, A_wo, B_x, B_k_cache, B_v_cache, B_wq, B_wo):
    ax = A_x.reshape(M, D); bx = B_x.reshape(M, D)
    bk = B_k_cache.reshape(B, G, 2 * SK, DH); bv = B_v_cache.reshape(B, G, 2 * SK, DH)
    hbm = pl.BlockSpec(memory_space=pltpu.HBM)
    out = pl.pallas_call(
        kernel,
        in_specs=[hbm] * 10,
        out_specs=hbm,
        out_shape=jax.ShapeDtypeStruct((M, 2*D), bf16),
        scratch_shapes=[
            pltpu.VMEM((2, M, D), bf16),
            pltpu.VMEM((2 * G, D, GW), bf16),
            pltpu.VMEM((2 * G - 1, D, GW), bf16),
            pltpu.VMEM((NP, GW), bf16),
            pltpu.VMEM((32 + 2 * NBS, 2 * SK, DH), bf16),
            pltpu.VMEM((32 + 2 * NBS, 2 * SK, DH), bf16),
            pltpu.VMEM((2 * D, M), f32),
            pltpu.VMEM((M, 2 * D), f32),
            pltpu.VMEM((M, GW), bf16),
            pltpu.VMEM((M, 2 * D), bf16),
            pltpu.SemaphoreType.DMA((NSEM,)),
        ],
        compiler_params=pltpu.CompilerParams(vmem_limit_bytes=110*1024*1024, disable_bounds_checks=True,
                                             disable_semaphore_checks=True),
    )(ax, A_k_cache, A_v_cache, A_wq, A_wo.T, bx, bk, bv, B_wq, B_wo.T)
    return out.reshape(B, SQ, 2*D)
```

```python
import jax
import jax.numpy as jnp
import jax.experimental.pallas as pl
import jax.experimental.pallas.tpu as pltpu

B, SQ, D, SK, DH = 8, 112, 448, 512, 256
M = B * SQ
G = 8
GW = 2 * DH
NP = 512
C0 = 2 * D - NP
QSCALE = DH ** -0.5
NBS = 16
V2LO = 12
VFLO = 13

ORD_V1 = ("W:q,o,k0,v0,k1,v1,k2,v2,k3,v3 Q0 Q1 S0 S1 S2 S3 P0 P1 P2 P3 I0 "
          "Q2 Q3 T0 S4 S5 S6 S7 P4 P5 P6 P7 I1 Q4 Q5 T1 T2 S8 S9 S10 S11 P8 P9 P10 P11 I2 "
          "Q6 Q7 T3 S12 S13 S14 S15 P12 P13 P14 P15 I3 T4 T5 T6").split()
ORD_V2 = ("W:q,o,k0,v0,k1,v1 Q0 Q1 X0 S0 S1 S2 S3 P0 P1 P2 P3 I0 "
          "Q2 Q3 T0 X1 S4 S5 S6 S7 P4 P5 P6 P7 I1 "
          "W:k2,v2,k3,v3 Q4 Q5 T1 T2 X2 S8 S9 S10 S11 P8 P9 P10 P11 I2 "
          "Q6 Q7 T3 X3 S12 S13 S14 S15 P12 P13 P14 P15 I3 T4 T5 T6").split()
ORD_VF = ("W:q,x Q0 Q1 Q2 Q3 W:k0,v0 Q4 S0 S1 S2 S3 P0 P1 P2 P3 I0 "
          "W:k1,v1,o Q5 T0 S4 S5 S6 S7 P4 P5 P6 P7 I1 "
          "W:k2,v2 Q6 T1 T2 S8 S9 S10 S11 P8 P9 P10 P11 I2 "
          "W:k3,v3 Q7 T3 S12 S13 S14 S15 P12 P13 P14 P15 I3 T4 T5 T6").split()

bf16 = jnp.bfloat16
f32 = jnp.float32

S_XA = 0
S_XB = 2
S_W = 3
S_KV = S_W + 32
S_VLAST = S_KV + 2 * (32 + NBS)
S_O = S_VLAST + 1
NSEM = S_O + 3


def _dot_nn(a, b):
    return jnp.dot(a, b, preferred_element_type=f32)


def _dot_nt(a, b):
    return jax.lax.dot_general(a, b, (((1,), (1,)), ((), ())), preferred_element_type=f32)


def _softmax_parts(s):
    m = jnp.max(s, axis=-1, keepdims=True)
    p = jnp.exp(s - m)
    l = jnp.sum(p, axis=-1, keepdims=True)
    r = pl.reciprocal(l, approx=True)
    r = r * (2.0 - l * r)
    return p.astype(bf16), r


def _static(x):
    return isinstance(x, (int, bool))


def _and(a, b):
    if _static(a):
        return b if a else False
    if _static(b):
        return a if b else False
    return jnp.logical_and(a, b)


def _sel(c, a, b):
    if _static(c):
        return a if c else b
    return jnp.where(c, a, b)


def _when(cond, fn):
    if _static(cond):
        if cond:
            fn()
    else:
        pl.when(cond)(fn)


def _mult(x, m):
    return x if _static(x) else pl.multiple_of(x, m)


def _kernel(ax, ak, av, awq, awo, bx, bk, bv, bwq, bwo, out,
            xbuf, wqbuf, wobuf, wolast, kbuf, vbuf, acc_t, acc_r, oscr, obuf, sem):
    def xa_copy(part):
        r = pl.ds(0, 2 * SQ) if part == 0 else pl.ds(2 * SQ, M - 2 * SQ)
        return pltpu.make_async_copy(ax.at[r], xbuf.at[0, r], sem.at[S_XA + part])

    def xb_copy():
        return pltpu.make_async_copy(bx, xbuf.at[1], sem.at[S_XB])

    def cols(j):
        return pl.ds(_mult(j * GW, GW), GW)

    def wq_copy(br, j):
        return pltpu.make_async_copy((awq, bwq)[br].at[:, cols(j)], wqbuf.at[br * G + j],
                                     sem.at[S_W + br * G + j])

    def wo_copy(br, j):
        if br == 1 and _static(j) and j == G - 1:
            dst = wolast.at[pl.ds(NP - D, D)]
        else:
            dst = wobuf.at[br * G + j]
        return pltpu.make_async_copy((awo, bwo)[br].at[:, cols(j)], dst,
                                     sem.at[S_W + 2 * G + br * G + j])

    def a_copies(j, bp):
        t = j * 4 + bp
        return [pltpu.make_async_copy(src.at[2 * bp + i, j], buf.at[t, pl.ds(i * SK, SK)],
                                      sem.at[S_KV + 2 * t + kv])
                for kv, (src, buf) in enumerate(((ak, kbuf), (av, vbuf))) for i in range(2)]

    def a_wait(j, bp, kv):
        t = j * 4 + bp
        buf = (kbuf, vbuf)[kv]
        pltpu.make_async_copy(buf.at[t], buf.at[t], sem.at[S_KV + 2 * t + kv]).wait()

    def b_copy(j, bp, kv, part=None):
        slot = (j * 4 + bp) & (NBS - 1)
        s0 = S_KV + 64 + 2 * slot + kv
        src, buf = ((bk, kbuf), (bv, vbuf))[kv]
        if part is None:
            return pltpu.make_async_copy(src.at[pl.ds(2 * bp, 2), j],
                                         buf.at[pl.ds(32 + 2 * slot, 2)], sem.at[s0])
        return pltpu.make_async_copy(src.at[2 * bp + part, j], buf.at[32 + 2 * slot + part],
                                     sem.at[(s0, S_VLAST)[part]])

    def b_copies(j, bp):
        if _static(j) and j == G - 1 and bp == 3:
            return [b_copy(j, bp, 0), b_copy(j, bp, 1, 0), b_copy(j, bp, 1, 1)]
        return [b_copy(j, bp, 0), b_copy(j, bp, 1)]

    def o_copy(k):
        r = pl.ds(0, 6 * SQ) if k == 0 else pl.ds((k + 5) * SQ, SQ)
        return pltpu.make_async_copy(obuf.at[r], out.at[r], sem.at[S_O + k])

    def issue_pkg(gi, bp, ok):
        first = bp == 0
        j = gi & (G - 1)

        def fa():
            if first:
                wq_copy(0, j).start()
            for c in a_copies(j, bp):
                c.start()
            if first:
                wo_copy(0, j).start()

        def fb(j):
            if first:
                wq_copy(1, j).start()
            for c in b_copies(j, bp):
                c.start()
            if first:
                wo_copy(1, j).start()

        _when(_and(ok, gi < G), fa)
        if first:
            _when(_and(ok, gi == G), lambda: xb_copy().start())
        if bp in (1, 2):
            _when(_and(ok, gi >= G), lambda: fb(j))
        else:
            _when(_and(ok, _and(gi >= G, gi < 2 * G - 1)), lambda: fb(j))
            _when(_and(ok, gi == 2 * G - 1), lambda: fb(G - 1))

    def issue(gi, k):
        for c in range(2):
            p = 4 + 2 * k + c
            g = 2 * gi + p // 4
            issue_pkg(g, p % 4, g < G + NBS // 4)
        g = gi + NBS // 4
        issue_pkg(g, k, _and(gi >= G, g < 2 * G))

    def waits(gi, items):
        j = gi & (G - 1)

        def w(br):
            for it in items:
                if it == "q":
                    wq_copy(br, j).wait()
                elif it == "o":
                    wo_copy(br, j).wait()
                elif it != "x":
                    kv, bp = "kv".index(it[0]), int(it[1])
                    if br == 0:
                        a_wait(j, bp, kv)
                    else:
                        b_copy(j, bp, kv).wait()

        if "q" in items:
            _when(gi == 0, lambda: xa_copy(0).wait())
            _when(gi == G, lambda: xb_copy().wait())
        if "x" in items:
            _when(gi == 0, lambda: xa_copy(1).wait())
        _when(gi < G, lambda: w(0))
        _when(gi >= G, lambda: w(1))

    def rows(b):
        return pl.ds(b * SQ, SQ)

    def qproj(gi, b):
        return (_dot_nn(xbuf[gi >> 3, rows(b), :], wqbuf[gi]) * QSCALE).astype(bf16)

    def kv_block(buf, gi, b, h):
        is_a = gi < G
        t = (gi & (G - 1)) * 4 + b // 2
        pair = _sel(is_a, t, 32 + 2 * (t & (NBS - 1)) + b % 2)
        half = _sel(is_a, b % 2, h)
        return buf[pair, pl.ds(_mult(half * SK, SK), SK), :]

    def s_head(gi, k, q):
        b, h = k // 2, k % 2
        return _softmax_parts(_dot_nt(q[:, h * DH:(h + 1) * DH], kv_block(kbuf, gi, b, h)))

    def p_head(gi, k, sm):
        return (_dot_nn(sm[0], kv_block(vbuf, gi, k // 2, k % 2)) * sm[1]).astype(bf16)

    def oproj_t(gi, n):
        c = slice(n * 128, (n + 1) * 128)
        r = pl.ds(_mult((gi >> 3) * D, 8), D)
        acc_t[r, c] += _dot_nt(wobuf[gi], oscr[c, :])

    def xpose(n, mlo, mhi):
        acc_r[n * 128:(n + 1) * 128, mlo * 128:mhi * 128] = (
            acc_t[mlo * 128:mhi * 128, n * 128:(n + 1) * 128].T)

    def group(gi, order):
        q, sm = {}, {}
        for st in order:
            kind = st[0]
            if kind == "W":
                waits(gi, st[2:].split(","))
                continue
            k = int(st[1:])
            if kind == "Q":
                q[k] = qproj(gi, k)
            elif kind == "S":
                sm[k] = s_head(gi, k, q[k // 2])
            elif kind == "P":
                oscr[rows(k // 2), (k % 2) * DH:(k % 2 + 1) * DH] = p_head(gi, k, sm[k])
            elif kind == "T":
                oproj_t(gi, k)
            elif kind == "I":
                issue(gi, k)
            elif kind == "X":
                for n in ((0, 1), (2, 3), (4, 5), (6,))[k]:
                    xpose(n, 0, 3)

    xa_copy(0).start()
    wq_copy(0, 0).start()
    xa_copy(1).start()
    for bp in range(4):
        for c in a_copies(0, bp):
            c.start()
        if bp == 1:
            wo_copy(0, 0).start()
    wolast[0:NP - D, :] = jnp.zeros((NP - D, GW), bf16)
    acc_t[...] = jnp.zeros_like(acc_t)

    def body(gi, carry):
        vf = jnp.logical_or(gi == 0, gi >= VFLO)
        v2 = jnp.logical_and(jnp.logical_not(vf), jnp.logical_or(gi == 1, gi >= V2LO))
        v1 = jnp.logical_not(jnp.logical_or(vf, v2))
        pl.when(vf)(lambda: group(gi, ORD_VF))
        pl.when(v2)(lambda: group(gi, ORD_V2))
        pl.when(v1)(lambda: group(gi, ORD_V1))
        return carry

    jax.lax.fori_loop(0, 2 * G - 1, body, 0)

    gi = 2 * G - 1

    def attend(b, sm):
        return jnp.concatenate([p_head(gi, 2 * b + h, sm[2 * b + h]) for h in range(2)], axis=1)

    def emit(b, o):
        r = rows(b)
        obuf[r, 0:C0] = acc_r[r, 0:C0].astype(bf16)
        obuf[r, C0:2 * D] = (acc_r[r, C0:2 * D] + _dot_nt(o, wolast[...])).astype(bf16)

    wq_copy(1, G - 1).wait()
    q = []
    for b in range(B):
        q.append(qproj(gi, b))
        if b < M // 128:
            xpose(b, 3, 7)
    sm = {}
    for bp in range(4):
        cs = b_copies(G - 1, bp)
        cs[0].wait()
        cs[1].wait()
        if bp == 0:
            wo_copy(1, G - 1).wait()
        if bp == 3:
            o_copy(0).start()
        for k in range(4 * bp, 4 * bp + 4):
            sm[k] = s_head(gi, k, q[k // 2])
        if bp < 3:
            o = [attend(2 * bp + i, sm) for i in range(2)]
            for i in range(2):
                emit(2 * bp + i, o[i])
        else:
            emit(2 * bp, attend(2 * bp, sm))
            o_copy(1).start()
            cs[2].wait()
            emit(2 * bp + 1, attend(2 * bp + 1, sm))
            o_copy(2).start()
    for k in range(3):
        o_copy(k).wait()


@jax.jit
def pallas_concat_heads__gqa_block_cached__mha_block_cached__near_ridge_kernel(
    A_x: jax.Array,
    A_k_cache: jax.Array,
    A_v_cache: jax.Array,
    A_wq: jax.Array,
    A_wo: jax.Array,
    B_x: jax.Array,
    B_k_cache: jax.Array,
    B_v_cache: jax.Array,
    B_wq: jax.Array,
    B_wo: jax.Array,
):
    hbm = pl.BlockSpec(memory_space=pltpu.HBM)
    out = pl.pallas_call(
        _kernel,
        in_specs=[hbm] * 10,
        out_specs=hbm,
        out_shape=jax.ShapeDtypeStruct((M, 2 * D), bf16),
        scratch_shapes=[
            pltpu.VMEM((2, M, D), bf16),
            pltpu.VMEM((2 * G, D, GW), bf16),
            pltpu.VMEM((2 * G - 1, D, GW), bf16),
            pltpu.VMEM((NP, GW), bf16),
            pltpu.VMEM((32 + 2 * NBS, 2 * SK, DH), bf16),
            pltpu.VMEM((32 + 2 * NBS, 2 * SK, DH), bf16),
            pltpu.VMEM((2 * D, M), f32),
            pltpu.VMEM((M, 2 * D), f32),
            pltpu.VMEM((M, GW), bf16),
            pltpu.VMEM((M, 2 * D), bf16),
            pltpu.SemaphoreType.DMA((NSEM,)),
        ],
        compiler_params=pltpu.CompilerParams(
            vmem_limit_bytes=110 * 1024 * 1024,
            disable_bounds_checks=True,
            disable_semaphore_checks=True,
        ),
    )(
        A_x.reshape(M, D), A_k_cache, A_v_cache, A_wq, A_wo.T,
        B_x.reshape(M, D), B_k_cache.reshape(B, G, 2 * SK, DH),
        B_v_cache.reshape(B, G, 2 * SK, DH), B_wq, B_wo.T,
    )
    return out.reshape(B, SQ, 2 * D)
```
